```python
import os as _os
_os.environ.setdefault("JAX_PLATFORMS", "cpu")
import jax
import jax.numpy as jnp

def _softmax(x, axis=-1):
    return jax.nn.softmax(x, axis=axis)
def _gelu(x):
    return jax.nn.gelu(x, approximate=True)
def _silu(x):
    return jax.nn.silu(x)
def _sigmoid(x):
    return jax.nn.sigmoid(x)
def _layernorm(x, axis=-1, eps=1e-5):
    m = jnp.mean(x, axis=axis, keepdims=True)
    v = jnp.var(x, axis=axis, keepdims=True)
    return (x - m) / jnp.sqrt(v + eps)
def _scatter_add(tgt, idx, src, axis=0):
    return tgt.at[idx].add(src)
def _segment_sum(src, seg, n):
    return jax.ops.segment_sum(src, seg, n)
class _Rng:
    def __init__(self, key):
        self._k = key
    def _next(self):
        self._k, sub = jax.random.split(self._k)
        return sub
    def normal(self, shape):
        return jax.random.normal(self._next(), shape, dtype=jnp.bfloat16)
    def randint(self, lo, hi, shape):
        return jax.random.randint(self._next(), shape, lo, hi, dtype=jnp.int32)
    def uniform(self, shape, lo=0.0, hi=1.0):
        return jax.random.uniform(self._next(), shape, jnp.bfloat16, lo, hi)
    def permutation(self, n):
        return jax.random.permutation(self._next(), n)


kernel_name = 'sequential_preLN__ssm_conv_h3__mixer_channel_mlp__prompt'

def setup_inputs():
    _rng = _Rng(jax.random.key(int.from_bytes(__import__("os").urandom(4), "little")))
    _w = (lambda a: (lambda t: t.astype(jnp.bfloat16) if jnp.issubdtype(t.dtype, jnp.floating) else t)(jnp.asarray(a)))
    def _A_setup():
        B, S, D = 1, 2048, 448
        ks = 4
        return {
            "q": _w((lambda *s: _rng.normal(s) * 0.05)(B, S, D)),
            "k": _w((lambda *s: _rng.normal(s) * 0.05)(B, S, D)),
            "v": _w((lambda *s: _rng.normal(s) * 0.05)(B, S, D)),
            "shift_k": _w((lambda *s: _rng.normal(s) * 0.05)(D, ks) * 0.5),
            "ssm_k": _w((lambda *s: _rng.normal(s) * 0.05)(D, S) * (1.0 / S ** 0.5)),
            "ssm_D": _w((lambda *s: _rng.normal(s) * 0.05)(D)),
        }
    _A_in = _A_setup()

    def _B_setup():
        B, S, D, F = 1, 2048, 448, 1792
        return {
            "x": _w((lambda *s: _rng.normal(s) * 0.05)(B, S, D)),
            "w1": _w((lambda *s: _rng.normal(s) * 0.2)(D, F) * (D ** -0.5)),
            "b1": _w((lambda *s: _rng.normal(s) * 0.2)(F)),
            "w2": _w((lambda *s: _rng.normal(s) * 0.2)(F, D) * (F ** -0.5)),
            "b2": _w((lambda *s: _rng.normal(s) * 0.05)(D)),
        }
    _B_in = _B_setup()

    return {
        "A_q": _A_in["q"],
        "A_k": _A_in["k"],
        "A_v": _A_in["v"],
        "A_shift_k": _A_in["shift_k"],
        "A_ssm_k": _A_in["ssm_k"],
        "A_ssm_D": _A_in["ssm_D"],
        "B_x": _B_in["x"],
        "B_w1": _B_in["w1"],
        "B_b1": _B_in["b1"],
        "B_w2": _B_in["w2"],
        "B_b2": _B_in["b2"],
    }

def reference(A_q, A_k, A_v, A_shift_k, A_ssm_k, A_ssm_D, B_x, B_w1, B_b1, B_w2, B_b2):
    def _A_ref(q, k, v, shift_k, ssm_k, ssm_D):
        B, S, D = q.shape
        ks = shift_k.shape[-1]
        k_pad = jnp.pad(k, ((0, 0), (ks - 1, 0), (0, 0)))
        k_shift = jnp.zeros_like(k)
        for t in range(ks):
            k_shift = k_shift + k_pad[:, t:t + S, :] * shift_k[:, ks - 1 - t][None, None, :]
        kv = k_shift * v
        L = 2 * S
        kv_pad = jnp.pad(kv, ((0, 0), (0, S), (0, 0)))
        kf_pad = jnp.pad(ssm_k, ((0, 0), (0, S)))
        kv_f = (lambda x, axes=(-2,-1): jnp.fft.rfft2(x.astype(jnp.float32), axes=axes))(kv_pad[:, None, :, :], axes=(1, 2))
        kf_f = (lambda x, axes=(-2,-1): jnp.fft.rfft2(x.astype(jnp.float32), axes=axes))(kf_pad[:, None, :], axes=(1, 2))
        kf_f = (lambda x, *d: x.transpose(*d))(kf_f, 1, 2, 0)
        y_f = kv_f * kf_f[None, :, :, :]
        y = (lambda x, s, axes=(-2,-1): jnp.fft.irfft2(x, s=s, axes=axes).astype(jnp.bfloat16))(y_f, (1, L), axes=(1, 2))[:, 0, :S, :]
        y = y + kv * ssm_D[None, None, :]
        return q * y

    def _B_ref(x, w1, b1, w2, b2):
        y = _layernorm(x, axis=-1)
        h = _gelu(jnp.einsum("bsd,df->bsf", y, w1) + b1)
        return jnp.einsum("bsf,fd->bsd", h, w2) + b2

    x = A_q
    h = x + _A_ref(_layernorm(x, axis=-1), A_k, A_v, A_shift_k, A_ssm_k, A_ssm_D)
    h2 = h + _B_ref(_layernorm(h, axis=-1), B_w1, B_b1, B_w2, B_b2)
    return h2
```

```python
import functools
import numpy as np
import jax
import jax.numpy as jnp
import jax.experimental.pallas as pl
import jax.experimental.pallas.tpu as pltpu

S, D, F = 2048, 448, 1792
T = 256
NT = S // T
B = 128
EPS = 1e-5
f32 = jnp.float32
bf16 = jnp.bfloat16
u32 = jnp.uint32

def _dft_matrix():
    n = np.arange(256)[:, None].astype(np.float64)
    k = np.arange(128)[None, :].astype(np.float64)
    th = 2 * np.pi * (k + 0.5) * n / 256
    return np.concatenate([np.cos(th), -np.sin(th)], axis=1).astype(np.float32)

NT_DIMS = (((1,), (1,)), ((), ()))
C0 = float(np.sqrt(2.0 / np.pi))
C1 = C0 * 0.044715


def _kernel(q_hbm, k_hbm, v_hbm, ssm_hbm, w1_hbm, w2_hbm, g_hbm, sh_hbm, d_hbm, b1_hbm, b2_hbm,
            o_ref,
            q_ref, k_ref, v_ref, ssm_ref, w1_ref, w2_ref, g_ref, sh_ref, d_ref, b1_ref, b2_ref,
            sem, ssem, z_ref,
            par_ref, w_ref, h_ref, b1b_ref, gu_ref, w1u_ref, w2u_ref,
            xs_ref, ks_ref, lraw_ref, kvb_ref, yn_ref, hres_ref):
    s = pl.program_id(0)
    srcs = (q_hbm, k_hbm, v_hbm, ssm_hbm)
    dsts = (q_ref, k_ref, v_ref, ssm_ref)
    zbox = []
    Q, K_, V_, SS, W1, W2 = range(6)

    def cp(a, t):
        if a < 4:
            return pltpu.make_async_copy(srcs[a].at[:, pl.ds(t * T, T)], dsts[a].at[t], sem.at[a, t])
        src, dst = ((w1_hbm, w1_ref), (w2_hbm, w2_ref))[a - 4]
        return pltpu.make_async_copy(src.at[:, pl.ds(t * 256, 256)], dst.at[:, pl.ds(t * 256, 256)], sem.at[a, t])

    def start(lst):
        for a, t in lst:
            cp(a, t).start()

    def wait(lst):
        for a, t in lst:
            cp(a, t).wait()

    pk = lambda x: pltpu.bitcast(x.astype(bf16), u32)
    upk = lambda x: pltpu.bitcast(x, bf16)
    gblk = lambda b: upk(gu_ref[b * 64:(b + 1) * 64, :])
    fmask = lambda: jax.lax.broadcasted_iota(jnp.int32, (8, B), 1) < zbox[0]
    def sel(dep, x):
        return x if dep is None else jnp.where(fmask(), dep, x)

    def dft(a):
        out = []
        for b in range(2):
            z = jnp.dot(a[:, b * B:(b + 1) * B], gblk(b), preferred_element_type=f32)
            out.append((z[:, :B], z[:, B:]))
        return out

    def KD(t):
        (c0, d0), (c1, d1) = dft(ssm_ref[t])
        if t == 0:
            c0 = c0 + par_ref[4]
        for i, a in enumerate((c0, d0, c1, d1)):
            lraw_ref[t % 3, i] = a

    def KPpos(t, r0, rc, link, chain=True):
        rows = slice(r0, r0 + rc)
        c0, d0, c1, d1 = (lraw_ref[t % 3, i, rows, :] for i in range(4))
        if t > 0:
            pc0, pd0, pc1, pd1 = (lraw_ref[(t - 1) % 3, i, rows, :] for i in range(4))
        else:
            pc0 = pd0 = pc1 = pd1 = None
        for p, (cc, pc, dd, pd, sg) in enumerate(((c0, pc1, d0, pd1, -1), (c0, pc0, d0, pd0, 1), (c1, pc1, d1, pd1, 1))):
            cc = sel(link, cc)
            if pc is None:
                c, d = cc, dd
            else:
                c = cc + pc if sg > 0 else cc - pc
                d = dd + pd if sg > 0 else dd - pd
            e = d - c
            f = (sel(e, c) if chain else c) + d
            link = f if chain else None
            ks_ref[t, 3 * p + 0, rows, :] = c
            ks_ref[t, 3 * p + 1, rows, :] = e
            ks_ref[t, 3 * p + 2, rows, :] = f
        return link

    def KV(t, link=None, nkv=None, rc=16):
        lane = jax.lax.broadcasted_iota(jnp.int32, (rc // 2, B), 1)
        if link is not None:
            link = pltpu.bitcast(link, u32)
        links = [link] * (nkv or 1)
        n = 0
        for r0 in range(0, D, rc):
            rows = slice(r0, r0 + rc)
            kp = pltpu.bitcast(k_ref[t, rows, :], u32)
            if t == 0:
                prev = jnp.zeros((rc // 2, B), u32)
            else:
                prev = pltpu.bitcast(k_ref[t - 1, rows, B:2 * B], u32)
            v = v_ref[t, rows, :].astype(f32)
            cols = [prev, kp[:, :B], kp[:, B:]]
            for c in (1, 2):
                cur = sel(links[n % len(links)], cols[c])
                a = upk(cur).astype(f32) * par_ref[0, rows, :]
                for u in (1, 2, 3):
                    m = jnp.where(lane >= B - u, cols[c - 1], cur)
                    a = a + upk(pltpu.roll(m, u, 1)).astype(f32) * par_ref[u, rows, :]
                out = pk(a * v[:, (c - 1) * B:c * B])
                if nkv:
                    links[n % nkv] = out
                n += 1
                kvb_ref[t % 2, r0 // 2:(r0 + rc) // 2, (c - 1) * B:c * B] = out

    def XD(t):
        (a0, b0), (a1, b1) = dft(upk(kvb_ref[t % 2]))
        s0 = a0 + b0
        s1 = a1 + b1
        xcur = [s0 + s1, a0 + a1, b0 + b1, s1, a1, b1, s0, a0, b0]
        for j in range(9):
            xs_ref[t, j] = xcur[j]

    def MACpos(r0, rc, pairs, link, chain=True):
        rows = slice(r0, r0 + rc)
        terms = [(lambda j, u=u, d=d: xs_ref[u, j, rows, :] * ks_ref[d, j, rows, :]) for (u, d) in pairs]
        n = len(terms)
        sl = sel if chain else (lambda dep, x: x)
        def run(a, j, sign, first=0):
            for i in range(first, n):
                a = a + terms[i](j) if sign > 0 else a - terms[i](j)
            return a
        r0_ = run(sl(link, terms[0](0)), 0, 1, 1)
        p1r = run(r0_, 2, -1)
        p1i = run(sl(p1r, r0_), 1, 1)
        r3 = run(sl(p1i, terms[0](3)), 3, 1, 1)
        w0r = run(p1r - r3, 5, 1)
        w0i = run(sl(w0r, p1i - r3), 4, -1)
        r6 = run(sl(w0i, terms[0](6)), 6, 1, 1)
        w1r = run(p1r + r6, 8, -1)
        w1i = run(sl(w1r, p1i + r6), 7, 1)
        return jnp.concatenate([w0r, w0i, w1r, w1i], axis=1), w1i

    def MACchain(t, nch, kp_pre=None, kp_post=None):
        pairs = [(u, t - u) for u in range(t + 1)]
        links = [None] * nch
        pend = None
        for g, r0 in enumerate(range(0, D, 8)):
            l = links[g % nch]
            if kp_pre is not None:
                l = KPpos(kp_pre, r0, 8, l)
            w, l = MACpos(r0, 8, pairs, l)
            if kp_post is not None:
                l = KPpos(kp_post, r0, 8, l)
            links[g % nch] = l
            if g % 2 == 0:
                pend = w
            else:
                w_ref[(r0 - 8) // 2:(r0 + 8) // 2, :] = pk(jnp.concatenate([pend, w], axis=0))

    def ID():
        ys = []
        for b in range(2):
            ys.append(jax.lax.dot_general(upk(w_ref[:, 2 * b * B:2 * (b + 1) * B]), gblk(b), NT_DIMS,
                                          preferred_element_type=f32))
        return jnp.concatenate(ys, axis=1)

    def fold8(a):
        r = a[0:8]
        for i in range(8, a.shape[0], 8):
            r = r + a[i:i + 8]
        return r

    def stats(s1, s2):
        m = jnp.sum(s1, axis=0, keepdims=True) * (1.0 / D)
        e2 = jnp.sum(s2, axis=0, keepdims=True) * (1.0 / D)
        return m, jnp.maximum(e2 - m * m, 0.0)

    def join(arrs):
        tiles = []
        for a in arrs:
            a = pltpu.bitcast(a, u32)
            tiles += [a[i:i + 8, j:j + B] for i in range(0, a.shape[0], 8) for j in range(0, a.shape[1], B)]
        d = tiles[0]
        for x in tiles[1:]:
            d = d | x
        return d

    def LN_all(t, y):
        s1 = s2 = None
        for r0 in range(0, D, 64):
            x = q_ref[t, r0:r0 + 64, :].astype(f32)
            a, b = fold8(x), fold8(x * x)
            s1 = a if s1 is None else s1 + a
            s2 = b if s2 is None else s2 + b
            yield join([s1, s2])
        m, var = stats(s1, s2)
        rq = jax.lax.rsqrt(var + EPS) * (1.0 / 128.0)
        mq = m * rq
        y = y()
        s1 = s2 = None
        for r0 in range(0, D, 32):
            rows = slice(r0, r0 + 32)
            x = q_ref[t, rows, :].astype(f32)
            h = x + (x * rq - mq) * y[rows]
            h_ref[rows, :] = h
            b2 = par_ref[5, rows, :]
            hres_ref[t % 2, rows, :] = (h + h) + jnp.concatenate([b2, b2], axis=1)
            a, b = fold8(h), fold8(h * h)
            s1 = a if s1 is None else s1 + a
            s2 = b if s2 is None else s2 + b
        yield None
        mh, vh = stats(s1, s2)
        rh = jax.lax.rsqrt(vh + EPS)
        mrh = mh * rh
        mz = mh * rh - mrh
        vz = vh * (rh * rh)
        rz = jax.lax.rsqrt(vz + EPS)
        A = rh * rz
        Bc = (mrh + mz) * rz
        for c in range(2):
            for r0 in range(0, D, B):
                rc2 = min(B, D - r0)
                hv = h_ref[pl.ds(pl.multiple_of(r0 + zbox[0], 8), rc2), c * B:(c + 1) * B]
                yn = hv * A[:, c * B:(c + 1) * B] - Bc[:, c * B:(c + 1) * B]
                yt = yn.astype(bf16).T
                yn_ref[t % 2, c * 64:(c + 1) * 64, r0:r0 + rc2] = pltpu.bitcast(yt, u32)
                if rc2 < B:
                    yt = jnp.concatenate([yt, yt], axis=1)
                yield join([yt[0:16], yt[B - 16:B]])

    def attach(x, deps):
        if not deps:
            return x
        parts = []
        pos = 0
        for r in sorted(deps):
            if 16 * r > pos:
                parts.append(x[pos:16 * r])
            blk = x[16 * r:16 * r + 16]
            t0 = upk(sel(deps[r], pltpu.bitcast(blk[:, :B], u32)))
            parts.append(jnp.concatenate([t0, blk[:, B:]], axis=1))
            pos = 16 * r + 16
        if pos < x.shape[0]:
            parts.append(x[pos:])
        return jnp.concatenate(parts, axis=0)

    def M1(t, c, deps, yn=None):
        f0, f1 = c * B, (c + 1) * B
        if t == 0:
            wv = w1_ref[:, f0:f1]
            w1u_ref[:, f0:f1] = pltpu.bitcast(wv, u32)
        else:
            wv = upk(w1u_ref[:, f0:f1])
        if yn is None:
            yn = upk(yn_ref[t % 2])
        x = jnp.dot(attach(yn, deps), wv, preferred_element_type=f32)
        x = x + jnp.concatenate([b1b_ref[:, f0:f1]] * (x.shape[0] // 8), axis=0)
        th = jnp.tanh(x * (C0 + C1 * (x * x)))
        return x + x * th

    def M2(t, hh, c, acc, deps):
        if t == 0:
            wv = w2_ref[:, c * 256:(c + 1) * 256]
            w2u_ref[:, c * 256:(c + 1) * 256] = pltpu.bitcast(wv, u32)
        else:
            wv = upk(w2u_ref[:, c * 256:(c + 1) * 256])
        return acc + jax.lax.dot_general(attach(wv, deps), hh.astype(bf16), NT_DIMS, preferred_element_type=f32)

    DUR = {"a": 256, "b": 448, "I": 448, "X": 448, "K": 448}

    def run_seq(tm, seq, special, task_fn):
        startt = []
        tt = 0
        for op in seq:
            startt.append(tt)
            tt += DUR.get(op[0], 0)
        total = tt
        pts = [(startt[m] + 16 * r, m, r) for m, op in enumerate(seq) if op in ("a", "b") for r in range(16 if op == "a" else 28)]
        tasks = {}
        def place(fn, when):
            for (tp_, m, r) in pts:
                if tp_ >= when and (m, r) not in tasks:
                    tasks[(m, r)] = fn
                    return
            raise ValueError
        def spread(fl, t0, t1):
            n = len(fl)
            for k, d in enumerate(fl):
                place(d, t0 + (t1 - t0) * (k + 1) / n)
        task_fn(lambda op: startt[seq.index(op)], total, spread)
        hh = {}
        acc = None
        na = nb = 0
        for m, op in enumerate(seq):
            deps = {r: tasks[(mm, r)]() for (mm, r) in sorted(tasks) if mm == m}
            if op == "a":
                hh[na] = M1(tm, na, deps)
                na += 1
            elif op == "b":
                if acc is None:
                    acc = hres_ref[tm % 2]
                acc = M2(tm, jnp.concatenate([hh[2 * nb], hh[2 * nb + 1]], axis=1), nb, acc, deps)
                nb += 1
            else:
                special[op]()
        o_ref[...] = (acc * 0.5).astype(o_ref.dtype)

    B1 = [(K_, 0), (V_, 0), (SS, 0)]
    B2 = [(Q, 0), (W1, 0), (W1, 1), (W2, 0)]
    B3 = [(K_, 1), (V_, 1), (SS, 1), (W1, 2), (W2, 1), (W1, 3)]
    B4 = [(W2, 2), (W1, 4), (W2, 3), (W1, 5), (SS, 2), (Q, 1)]
    B5 = [(W2, 4), (W1, 6), (W2, 5), (W2, 6), (K_, 2), (V_, 2)]
    B6 = [(SS, 3), (Q, 2), (K_, 3), (V_, 3), (SS, 4)]

    def step0():
        small = [pltpu.make_async_copy(a, b, sem.at[6, i]) for i, (a, b) in enumerate(
            ((sh_hbm, sh_ref), (d_hbm, d_ref), (b2_hbm, b2_ref), (b1_hbm, b1_ref), (g_hbm, g_ref)))]
        for c in small:
            c.start()
        start(B1 + B2 + B3 + B4 + B5 + B6)
        z_ref[0] = 0
        for c in small:
            c.wait()
        col = lambda r: jnp.broadcast_to(r, (B, D)).T
        sh = sh_ref[...].astype(f32)
        for u in range(4):
            par_ref[u] = col(sh[u:u + 1])
        par_ref[4] = col(d_ref[...].reshape(1, D).astype(f32))
        par_ref[5] = col(b2_ref[...].reshape(1, D).astype(f32) * 2.0)
        gu_ref[...] = pltpu.bitcast(g_ref[...], u32)
        b1b_ref[...] = jnp.broadcast_to(b1_ref[...].reshape(1, F).astype(f32), (8, F))
        wait(B1)
        KD(0)
        KV(0, rc=D)
        XD(0)
        for r0 in range(0, D, 32):
            KPpos(0, r0, 32, None, chain=False)
            w, _ = MACpos(r0, 32, [(0, 0)], None, chain=False)
            w_ref[r0 // 2:(r0 + 32) // 2, :] = pk(w)

    def step1():
        zbox[:] = [z_ref[0]]
        ybox = []
        ln1 = LN_all(1, lambda: ybox[0])
        def ln0():
            y = ID()
            for _ in LN_all(0, lambda: y):
                pass
        def i1():
            for _ in range(7):
                next(ln1)
            ybox.append(ID())
            next(ln1)
        special = {
            "w2": lambda: wait(B2),
            "I0": ln0,
            "w3": lambda: wait(B3),
            "K1": lambda: KD(1),
            "X1": lambda: (KV(1, None, 6), XD(1)),
            "w4": lambda: wait(B4),
            "K2": lambda: (MACchain(1, 2, kp_pre=1), KD(2)),
            "w5": lambda: wait(B5),
            "I1": i1,
            "e": lambda: (KV(2, ybox[0][D - 8:D, 0:B], 8), KPpos(2, 0, D, None, chain=False)),
        }
        seq = "w2 I0 a a a a b w3 K1 a a b a a X1 w4 b a a b a a K2 w5 I1 b a a b b e".split()
        def tk(st, total, spread):
            tA = st("I1") + 448
            spread([lambda: next(ln1)] * 8, tA + 500, min(tA + 1000, total - 150))
        run_seq(0, seq, special, tk)

    def step(t):
        zbox[:] = [z_ref[0]]
        nxt = t + 1 < NT
        hasK = t + 2 < NT
        need = [(Q, t)] + ([(K_, t + 1), (V_, t + 1)] if nxt else []) + ([(SS, t + 2)] if hasK else [])
        if t == 2:
            need = B6
        wait(need)
        start([(a, tt) for a, tt in ((Q, t + 1), (K_, t + 2), (V_, t + 2), (SS, t + 3)) if tt < NT])
        base = "a a a a b a a b a a b a a b a a b a a b b".split()
        nch = 2
        t_mac = 100 + 56 / nch * (18 * (t + 1) + 14 + (24 if nxt else 0)) * 1.05 - (448 if hasK else 0)
        tt = 0
        pos = len(base)
        for m, op in enumerate(base):
            if tt >= t_mac:
                pos = m
                break
            tt += DUR[op]
        seq = (["K3"] if t == 2 else []) + ["X"] + base[:pos] + ["M"] + (["K"] if hasK else []) + ["I"] + base[pos:] + ["e"]
        ybox = []
        ln = LN_all(t, lambda: ybox[0])
        info = {}
        def tk(st, total, spread):
            tI = st("I")
            tA = tI + 448
            lnext = lambda: next(ln)
            spread([lnext] * 7, st("X") + 448, tI - 100 - (448 if hasK else 0))
            spread([lnext] * 8, tA + 500, min(tA + 1000, total - 150))
            info["left"] = total - tA - 1000
        def fin():
            if nxt:
                nkv = max(4, min(8, int(np.ceil(56 * 135 / max(info["left"], 1)))))
                KV(t + 1, ybox[0][D - 8:D, 0:B], nkv)
        special = {
            "K3": lambda: KD(3),
            "X": lambda: XD(t),
            "M": lambda: MACchain(t, nch, kp_post=t + 1 if nxt else None),
            "K": lambda: KD(t + 2),
            "I": lambda: (ybox.append(ID()), next(ln)),
            "e": fin,
        }
        run_seq(t - 1, seq, special, tk)

    def last_step():
        t = NT - 1
        def body(hf, carry):
            col = pl.ds(pl.multiple_of(hf * B, B), B)
            yn = upk(yn_ref[t % 2, pl.ds(pl.multiple_of(hf * 64, 64), 64), :])
            acc = hres_ref[t % 2, :, col]
            hh = {}
            order = "a a a a a a a a b a a a a b a a b b".split()
            na = nb = 0
            for op in order:
                if op == "a":
                    hh[na] = M1(t, na, {}, yn)
                    na += 1
                else:
                    k0 = 4 * nb
                    k1 = min(k0 + 4, 14)
                    hcat = jnp.concatenate([hh[k] for k in range(k0, k1)], axis=1).astype(bf16)
                    wv = upk(w2u_ref[:, k0 * B:k1 * B])
                    acc = acc + jax.lax.dot_general(wv, hcat, NT_DIMS, preferred_element_type=f32)
                    nb += 1
            o_ref[:, col] = (acc * 0.5).astype(o_ref.dtype)
            return carry
        jax.lax.fori_loop(0, 2, body, 0)

    fns = [step0, step1] + [functools.partial(step, i) for i in range(2, NT)] + [last_step]
    for i, fn in enumerate(fns):
        pl.when(s == i)(fn)


@jax.jit
def pallas_sequential_preLN__ssm_conv_h3__mixer_channel_mlp__prompt_kernel(A_q, A_k, A_v, A_shift_k, A_ssm_k, A_ssm_D, B_x, B_w1, B_b1, B_w2, B_b2):
    qT = jnp.transpose(A_q[0])
    kT = jnp.transpose(A_k[0])
    vT = jnp.transpose(A_v[0])
    g = jnp.asarray(_dft_matrix(), dtype=bf16)
    anyspec = pl.BlockSpec(memory_space=pl.ANY)
    out = pl.pallas_call(
        _kernel,
        grid=(NT + 1,),
        in_specs=[anyspec] * 11,
        out_specs=pl.BlockSpec((D, T), lambda i: (0, jnp.maximum(i - 1, 0))),
        scratch_shapes=[
            pltpu.VMEM((NT, D, T), bf16),
            pltpu.VMEM((NT, D, T), bf16),
            pltpu.VMEM((NT, D, T), bf16),
            pltpu.VMEM((NT, D, T), bf16),
            pltpu.VMEM((D, F), bf16),
            pltpu.VMEM((D, F), bf16),
            pltpu.VMEM((256, 256), bf16),
            pltpu.VMEM((4, D), bf16),
            pltpu.VMEM((D,), bf16),
            pltpu.VMEM((F,), bf16),
            pltpu.VMEM((D,), bf16),
            pltpu.SemaphoreType.DMA((7, NT)),
            pltpu.SemaphoreType.DMA((5,)),
            pltpu.SMEM((1,), jnp.int32),
            pltpu.VMEM((6, D, B), f32),
            pltpu.VMEM((D // 2, 2 * T), u32),
            pltpu.VMEM((D, T), f32),
            pltpu.VMEM((8, F), f32),
            pltpu.VMEM((128, 256), u32),
            pltpu.VMEM((D // 2, F), u32),
            pltpu.VMEM((D // 2, F), u32),
            pltpu.VMEM((NT, 9, D, B), f32),
            pltpu.VMEM((NT, 9, D, B), f32),
            pltpu.VMEM((3, 4, D, B), f32),
            pltpu.VMEM((2, D // 2, T), u32),
            pltpu.VMEM((2, T // 2, D), u32),
            pltpu.VMEM((2, D, T), f32),
        ],
        out_shape=jax.ShapeDtypeStruct((D, S), bf16),
        compiler_params=pltpu.CompilerParams(
            dimension_semantics=("arbitrary",), vmem_limit_bytes=110 * 1024 * 1024),
        name="h3mlp",
    )(qT, kT, vT, A_ssm_k, B_w1, B_w2.T, g, A_shift_k.T, A_ssm_D, B_b1, B_b2)
    return out.T[None]
```

```python
import functools
import numpy as np
import jax
import jax.numpy as jnp
import jax.experimental.pallas as pl
import jax.experimental.pallas.tpu as pltpu

S, D, F = 2048, 448, 1792
T = 256
NT = S // T
B = 128
EPS = 1e-5
f32 = jnp.float32
bf16 = jnp.bfloat16
u32 = jnp.uint32

def _dft_matrix():
    n = np.arange(256)[:, None].astype(np.float64)
    k = np.arange(128)[None, :].astype(np.float64)
    th = 2 * np.pi * (k + 0.5) * n / 256
    return np.concatenate([np.cos(th), -np.sin(th)], axis=1).astype(np.float32)

NT_DIMS = (((1,), (1,)), ((), ()))
C0 = float(np.sqrt(2.0 / np.pi))
C1 = C0 * 0.044715


def _kernel(q_hbm, k_hbm, v_hbm, ssm_hbm, w1_hbm, w2_hbm, g_hbm, sh_hbm, d_hbm, b1_hbm, b2_hbm,
            o_ref,
            q_ref, k_ref, v_ref, ssm_ref, w1_ref, w2_ref, g_ref, sh_ref, d_ref, b1_ref, b2_ref,
            sem, z_ref,
            par_ref, w_ref, h_ref, b1b_ref, gu_ref, w1u_ref, w2u_ref,
            xs_ref, ks_ref, lraw_ref, kvb_ref, yn_ref, hres_ref):
    s = pl.program_id(0)
    srcs = (q_hbm, k_hbm, v_hbm, ssm_hbm)
    dsts = (q_ref, k_ref, v_ref, ssm_ref)
    zbox = []
    Q, K_, V_, SS, W1, W2 = range(6)

    def cp(a, t, si):
        if a < 4:
            return pltpu.make_async_copy(srcs[a].at[:, pl.ds(t * T, T)], dsts[a].at[t], sem.at[si])
        src, dst = ((w1_hbm, w1_ref), (w2_hbm, w2_ref))[a - 4]
        return pltpu.make_async_copy(src.at[:, pl.ds(t * 256, 256)], dst.at[:, pl.ds(t * 256, 256)], sem.at[si])

    def start(batch):
        for a, t in batch[1]:
            cp(a, t, batch[0]).start()

    def wait(batch):
        for a, t in batch[1]:
            cp(a, t, batch[0]).wait()

    pk = lambda x: pltpu.bitcast(x.astype(bf16), u32)
    upk = lambda x: pltpu.bitcast(x, bf16)
    gblk = lambda b: upk(gu_ref[b * 64:(b + 1) * 64, :])
    def sel(dep, x):
        if dep is None:
            return x
        return jnp.where(jax.lax.broadcasted_iota(jnp.int32, x.shape, 1) < zbox[0], dep, x)

    def dft(a):
        out = []
        for b in range(2):
            z = jnp.dot(a[:, b * B:(b + 1) * B], gblk(b), preferred_element_type=f32)
            out.append((z[:, :B], z[:, B:]))
        return out

    def KD(t):
        (c0, d0), (c1, d1) = dft(ssm_ref[t])
        if t == 0:
            c0 = c0 + par_ref[4]
        for i, a in enumerate((c0, d0, c1, d1)):
            lraw_ref[t % 3, i] = a

    def KPpos(t, r0, rc, link, chain=True):
        rows = slice(r0, r0 + rc)
        c0, d0, c1, d1 = (lraw_ref[t % 3, i, rows, :] for i in range(4))
        if t > 0:
            pc0, pd0, pc1, pd1 = (lraw_ref[(t - 1) % 3, i, rows, :] for i in range(4))
        else:
            pc0 = pd0 = pc1 = pd1 = None
        for p, (cc, pc, dd, pd, sg) in enumerate(((c0, pc1, d0, pd1, -1), (c0, pc0, d0, pd0, 1), (c1, pc1, d1, pd1, 1))):
            cc = sel(link, cc)
            if pc is None:
                c, d = cc, dd
            else:
                c = cc + pc if sg > 0 else cc - pc
                d = dd + pd if sg > 0 else dd - pd
            e = d - c
            f = (sel(e, c) if chain else c) + d
            link = f if chain else None
            ks_ref[t, 3 * p + 0, rows, :] = c
            ks_ref[t, 3 * p + 1, rows, :] = e
            ks_ref[t, 3 * p + 2, rows, :] = f
        return link

    def KV(t, link=None, nkv=None, rc=16):
        lane = jax.lax.broadcasted_iota(jnp.int32, (rc // 2, B), 1)
        if link is not None:
            link = pltpu.bitcast(link, u32)
        links = [link] * (nkv or 1)
        n = 0
        for r0 in range(0, D, rc):
            rows = slice(r0, r0 + rc)
            kp = pltpu.bitcast(k_ref[t, rows, :], u32)
            if t == 0:
                prev = jnp.zeros((rc // 2, B), u32)
            else:
                prev = pltpu.bitcast(k_ref[t - 1, rows, B:2 * B], u32)
            v = v_ref[t, rows, :].astype(f32)
            cols = [prev, kp[:, :B], kp[:, B:]]
            for c in (1, 2):
                cur = sel(links[n % len(links)], cols[c])
                a = upk(cur).astype(f32) * par_ref[0, rows, :]
                for u in (1, 2, 3):
                    m = jnp.where(lane >= B - u, cols[c - 1], cur)
                    a = a + upk(pltpu.roll(m, u, 1)).astype(f32) * par_ref[u, rows, :]
                out = pk(a * v[:, (c - 1) * B:c * B])
                if nkv:
                    links[n % nkv] = out
                n += 1
                kvb_ref[t % 2, r0 // 2:(r0 + rc) // 2, (c - 1) * B:c * B] = out

    def XD(t):
        (a0, b0), (a1, b1) = dft(upk(kvb_ref[t % 2]))
        s0 = a0 + b0
        s1 = a1 + b1
        xcur = [s0 + s1, a0 + a1, b0 + b1, s1, a1, b1, s0, a0, b0]
        for j in range(9):
            xs_ref[t, j] = xcur[j]

    def MACpos(r0, rc, pairs, link, chain=True):
        rows = slice(r0, r0 + rc)
        terms = [(lambda j, u=u, d=d: xs_ref[u, j, rows, :] * ks_ref[d, j, rows, :]) for (u, d) in pairs]
        n = len(terms)
        sl = sel if chain else (lambda dep, x: x)
        def run(a, j, sign, first=0):
            for i in range(first, n):
                a = a + terms[i](j) if sign > 0 else a - terms[i](j)
            return a
        r0_ = run(sl(link, terms[0](0)), 0, 1, 1)
        p1r = run(r0_, 2, -1)
        p1i = run(sl(p1r, r0_), 1, 1)
        r3 = run(sl(p1i, terms[0](3)), 3, 1, 1)
        w0r = run(p1r - r3, 5, 1)
        w0i = run(sl(w0r, p1i - r3), 4, -1)
        r6 = run(sl(w0i, terms[0](6)), 6, 1, 1)
        w1r = run(p1r + r6, 8, -1)
        w1i = run(sl(w1r, p1i + r6), 7, 1)
        return jnp.concatenate([w0r, w0i, w1r, w1i], axis=1), w1i

    def MACchain(t, nch, kp_pre=None, kp_post=None):
        pairs = [(u, t - u) for u in range(t + 1)]
        l = None
        for r0 in range(0, D, 16):
            if kp_pre is not None:
                l = KPpos(kp_pre, r0, 16, l)
            w, l = MACpos(r0, 16, pairs, l)
            if kp_post is not None:
                l = KPpos(kp_post, r0, 16, l)
            w_ref[r0 // 2:(r0 + 16) // 2, :] = pk(w)

    def ID():
        ys = []
        for b in range(2):
            ys.append(jax.lax.dot_general(upk(w_ref[:, 2 * b * B:2 * (b + 1) * B]), gblk(b), NT_DIMS,
                                          preferred_element_type=f32))
        return jnp.concatenate(ys, axis=1)

    def fold8(a):
        r = a[0:8]
        for i in range(8, a.shape[0], 8):
            r = r + a[i:i + 8]
        return r

    def stats(s1, s2):
        m = jnp.sum(s1, axis=0, keepdims=True) * (1.0 / D)
        e2 = jnp.sum(s2, axis=0, keepdims=True) * (1.0 / D)
        return m, jnp.maximum(e2 - m * m, 0.0)

    def join(arrs):
        tiles = []
        for a in arrs:
            a = pltpu.bitcast(a, u32)
            tiles += [a[i:i + 8, j:j + B] for i in range(0, a.shape[0], 8) for j in range(0, a.shape[1], B)]
        d = tiles[0]
        for x in tiles[1:]:
            d = d | x
        return d

    def LN_all(t, y):
        s1 = s2 = None
        for r0 in range(0, D, 64):
            x = q_ref[t, r0:r0 + 64, :].astype(f32)
            a, b = fold8(x), fold8(x * x)
            s1 = a if s1 is None else s1 + a
            s2 = b if s2 is None else s2 + b
            yield join([s1, s2])
        m, var = stats(s1, s2)
        rq = jax.lax.rsqrt(var + EPS) * (1.0 / 128.0)
        mq = m * rq
        y = y()
        s1 = s2 = None
        for r0 in range(0, D, 32):
            rows = slice(r0, r0 + 32)
            x = q_ref[t, rows, :].astype(f32)
            h = x + (x * rq - mq) * y[rows]
            h_ref[rows, :] = h
            b2 = par_ref[5, rows, :]
            hres_ref[t % 2, rows, :] = (h + h) + jnp.concatenate([b2, b2], axis=1)
            a, b = fold8(h), fold8(h * h)
            s1 = a if s1 is None else s1 + a
            s2 = b if s2 is None else s2 + b
        yield None
        mh, vh = stats(s1, s2)
        rh = jax.lax.rsqrt(vh + EPS)
        mrh = mh * rh
        mz = mh * rh - mrh
        vz = vh * (rh * rh)
        rz = jax.lax.rsqrt(vz + EPS)
        A = rh * rz
        Bc = (mrh + mz) * rz
        for c in range(2):
            for r0 in range(0, D, B):
                rc2 = min(B, D - r0)
                hv = h_ref[pl.ds(pl.multiple_of(r0 + zbox[0], 8), rc2), c * B:(c + 1) * B]
                yn = hv * A[:, c * B:(c + 1) * B] - Bc[:, c * B:(c + 1) * B]
                yt = yn.astype(bf16).T
                yn_ref[t % 2, c * 64:(c + 1) * 64, r0:r0 + rc2] = pltpu.bitcast(yt, u32)
                if rc2 < B:
                    yt = jnp.concatenate([yt, yt], axis=1)
                yield join([yt[0:16], yt[B - 16:B]])

    def attach(x, deps):
        if not deps:
            return x
        parts = []
        pos = 0
        for r in sorted(deps):
            if 16 * r > pos:
                parts.append(x[pos:16 * r])
            blk = x[16 * r:16 * r + 16]
            t0 = upk(sel(deps[r], pltpu.bitcast(blk[:, :B], u32)))
            parts.append(jnp.concatenate([t0, blk[:, B:]], axis=1))
            pos = 16 * r + 16
        if pos < x.shape[0]:
            parts.append(x[pos:])
        return jnp.concatenate(parts, axis=0)

    def M1(t, c, deps, yn=None):
        f0, f1 = c * B, (c + 1) * B
        if t == 0:
            wv = w1_ref[:, f0:f1]
            w1u_ref[:, f0:f1] = pltpu.bitcast(wv, u32)
        else:
            wv = upk(w1u_ref[:, f0:f1])
        if yn is None:
            yn = upk(yn_ref[t % 2])
        x = jnp.dot(attach(yn, deps), wv, preferred_element_type=f32)
        x = x + jnp.concatenate([b1b_ref[:, f0:f1]] * (x.shape[0] // 8), axis=0)
        th = jnp.tanh(x * (C0 + C1 * (x * x)))
        return x + x * th

    def M2(t, hh, c, acc, deps):
        if t == 0:
            wv = w2_ref[:, c * 256:(c + 1) * 256]
            w2u_ref[:, c * 256:(c + 1) * 256] = pltpu.bitcast(wv, u32)
        else:
            wv = upk(w2u_ref[:, c * 256:(c + 1) * 256])
        return acc + jax.lax.dot_general(attach(wv, deps), hh.astype(bf16), NT_DIMS, preferred_element_type=f32)

    DUR = {"a": 256, "b": 448, "I": 448, "X": 448, "K": 448}

    def run_seq(tm, seq, special, task_fn):
        startt = []
        tt = 0
        for op in seq:
            startt.append(tt)
            tt += DUR.get(op[0], 0)
        total = tt
        pts = [(startt[m] + 16 * r, m, r) for m, op in enumerate(seq) if op in ("a", "b") for r in range(16 if op == "a" else 28)]
        tasks = {}
        def place(fn, when):
            for (tp_, m, r) in pts:
                if tp_ >= when and (m, r) not in tasks:
                    tasks[(m, r)] = fn
                    return
            raise ValueError
        def spread(fl, t0, t1):
            n = len(fl)
            for k, d in enumerate(fl):
                place(d, t0 + (t1 - t0) * (k + 1) / n)
        task_fn(lambda op: startt[seq.index(op)], total, spread)
        hh = {}
        acc = None
        na = nb = 0
        for m, op in enumerate(seq):
            deps = {r: tasks[(mm, r)]() for (mm, r) in sorted(tasks) if mm == m}
            if op == "a":
                hh[na] = M1(tm, na, deps)
                na += 1
            elif op == "b":
                if acc is None:
                    acc = hres_ref[tm % 2]
                acc = M2(tm, jnp.concatenate([hh[2 * nb], hh[2 * nb + 1]], axis=1), nb, acc, deps)
                nb += 1
            else:
                special[op]()
        o_ref[...] = (acc * 0.5).astype(o_ref.dtype)

    B1 = (1, [(K_, 0), (V_, 0), (SS, 0)])
    BQ = (2, [(Q, 0)])
    B2 = (3, [(W1, 0), (W1, 1), (W2, 0)])
    B3 = (4, [(K_, 1), (V_, 1), (SS, 1), (W1, 2), (W2, 1), (W1, 3)])
    B4 = (5, [(W2, 2), (W1, 4), (W2, 3), (W1, 5), (SS, 2), (Q, 1)])
    B5 = (6, [(W2, 4), (W1, 6), (W2, 5), (W2, 6), (K_, 2), (V_, 2)])
    B6 = (7, [(SS, 3), (Q, 2), (K_, 3), (V_, 3), (SS, 4)])

    def step_batch(t):
        return (t % 2, [(a, tt) for a, tt in ((Q, t), (K_, t + 1), (V_, t + 1), (SS, t + 2)) if tt < NT])

    def step0():
        small = [pltpu.make_async_copy(a, b, sem.at[0]) for i, (a, b) in enumerate(
            ((sh_hbm, sh_ref), (d_hbm, d_ref), (b2_hbm, b2_ref), (b1_hbm, b1_ref), (g_hbm, g_ref)))]
        for c in small:
            c.start()
        for b in (B1, BQ, B2, B3, B4, B5, B6):
            start(b)
        z_ref[0] = 0
        for c in small:
            c.wait()
        col = lambda r: jnp.broadcast_to(r, (B, D)).T
        sh = sh_ref[...].astype(f32)
        for u in range(4):
            par_ref[u] = col(sh[u:u + 1])
        par_ref[4] = col(d_ref[...].reshape(1, D).astype(f32))
        par_ref[5] = col(b2_ref[...].reshape(1, D).astype(f32) * 2.0)
        gu_ref[...] = pltpu.bitcast(g_ref[...], u32)
        b1b_ref[...] = jnp.broadcast_to(b1_ref[...].reshape(1, F).astype(f32), (8, F))
        wait(B1)
        KD(0)
        KV(0, rc=D)
        XD(0)
        for r0 in range(0, D, 32):
            KPpos(0, r0, 32, None, chain=False)
            w, _ = MACpos(r0, 32, [(0, 0)], None, chain=False)
            w_ref[r0 // 2:(r0 + 32) // 2, :] = pk(w)

    def step1():
        zbox[:] = [z_ref[0]]
        ybox = []
        ln1 = LN_all(1, lambda: ybox[0])
        def ln0():
            y = ID()
            for _ in LN_all(0, lambda: y):
                pass
        special = {
            "wq": lambda: wait(BQ),
            "w2": lambda: wait(B2),
            "I0": ln0,
            "w3": lambda: wait(B3),
            "K1": lambda: (KD(1), KPpos(1, 0, D, None, chain=False)),
            "v1": lambda: KV(1, None, 6),
            "X1": lambda: XD(1),
            "w4": lambda: wait(B4),
            "K2": lambda: (MACchain(1, 2), KD(2)),
            "w5": lambda: wait(B5),
            "I1": lambda: (ybox.append(ID()), next(ln1)),
            "e": lambda: KV(2, ybox[0][D - 8:D, 0:B], 8),
        }
        seq = "wq I0 w2 a a a a b w3 K1 a a b a a v1 w4 X1 b a a b a a K2 w5 I1 b a a b b e".split()
        def tk(st, total, spread):
            tA = st("I1") + 448
            spread([lambda: next(ln1)] * 7, st("X1") + 448, st("K2") - 100)
            spread([lambda: next(ln1)] * 8, tA + 500, min(tA + 1000, total - 150))
        run_seq(0, seq, special, tk)

    def step(t):
        zbox[:] = [z_ref[0]]
        nxt = t + 1 < NT
        hasK = t + 2 < NT
        wait(B6 if t == 2 else step_batch(t))
        if nxt:
            start(step_batch(t + 1))
        base = "a a a a b a a b a a b a a b a a b a a b b".split()
        nch = 2
        t_mac = 100 + 56 / nch * (18 * (t + 1) + 14 + (24 if nxt else 0) + (24 if t == 2 else 0)) * 1.05 - (448 if hasK else 0)
        tt = 0
        pos = len(base)
        for m, op in enumerate(base):
            if tt >= t_mac:
                pos = m
                break
            tt += DUR[op]
        seq = (["K3"] if t == 2 else []) + ["X"] + base[:pos] + ["M"] + (["K"] if hasK else []) + ["I"] + base[pos:] + ["e"]
        ybox = []
        ln = LN_all(t, lambda: ybox[0])
        info = {}
        def tk(st, total, spread):
            tI = st("I")
            tA = tI + 448
            lnext = lambda: next(ln)
            spread([lnext] * 7, st("X") + 448, tI - 100 - (448 if hasK else 0))
            spread([lnext] * 8, tA + 500, min(tA + 1000, total - 150))
            info["left"] = total - tA - 1000
        def fin():
            if nxt:
                nkv = max(4, min(8, int(np.ceil(56 * 135 / max(info["left"], 1)))))
                KV(t + 1, ybox[0][D - 8:D, 0:B], nkv)
        special = {
            "K3": lambda: KD(3),
            "X": lambda: XD(t),
            "M": lambda: MACchain(t, nch, kp_pre=2 if t == 2 else None, kp_post=t + 1 if nxt else None),
            "K": lambda: KD(t + 2),
            "I": lambda: (ybox.append(ID()), next(ln)),
            "e": fin,
        }
        run_seq(t - 1, seq, special, tk)

    def last_step():
        t = NT - 1
        def body(hf, carry):
            col = pl.ds(pl.multiple_of(hf * B, B), B)
            yn = upk(yn_ref[t % 2, pl.ds(pl.multiple_of(hf * 64, 64), 64), :])
            acc = hres_ref[t % 2, :, col]
            hh = {}
            order = "a a a a a a a a b a a a a b a a b b".split()
            na = nb = 0
            for op in order:
                if op == "a":
                    hh[na] = M1(t, na, {}, yn)
                    na += 1
                else:
                    k0 = 4 * nb
                    k1 = min(k0 + 4, 14)
                    hcat = jnp.concatenate([hh[k] for k in range(k0, k1)], axis=1).astype(bf16)
                    if k1 - k0 == 4:
                        wv = upk(w2u_ref[:, k0 * B:k1 * B])
                        acc = acc + jax.lax.dot_general(wv, hcat, NT_DIMS, preferred_element_type=f32)
                    else:
                        parts = []
                        for m0 in (0, D // 2):
                            wv = upk(w2u_ref[m0 // 2:(m0 + D // 2) // 2, k0 * B:k1 * B])
                            parts.append(acc[m0:m0 + D // 2]
                                         + jax.lax.dot_general(wv, hcat, NT_DIMS, preferred_element_type=f32))
                        acc = jnp.concatenate(parts, axis=0)
                    nb += 1
            o_ref[:, col] = (acc * 0.5).astype(o_ref.dtype)
            return carry
        jax.lax.fori_loop(0, 2, body, 0)

    fns = [step0, step1] + [functools.partial(step, i) for i in range(2, NT)] + [last_step]
    for i, fn in enumerate(fns):
        pl.when(s == i)(fn)


@jax.jit
def pallas_sequential_preLN__ssm_conv_h3__mixer_channel_mlp__prompt_kernel(A_q, A_k, A_v, A_shift_k, A_ssm_k, A_ssm_D, B_x, B_w1, B_b1, B_w2, B_b2):
    qT = jnp.transpose(A_q[0])
    kT = jnp.transpose(A_k[0])
    vT = jnp.transpose(A_v[0])
    g = jnp.asarray(_dft_matrix(), dtype=bf16)
    anyspec = pl.BlockSpec(memory_space=pl.ANY)
    out = pl.pallas_call(
        _kernel,
        grid=(NT + 1,),
        in_specs=[anyspec] * 11,
        out_specs=pl.BlockSpec((D, T), lambda i: (0, jnp.maximum(i - 1, 0))),
        scratch_shapes=[
            pltpu.VMEM((NT, D, T), bf16),
            pltpu.VMEM((NT, D, T), bf16),
            pltpu.VMEM((NT, D, T), bf16),
            pltpu.VMEM((NT, D, T), bf16),
            pltpu.VMEM((D, F), bf16),
            pltpu.VMEM((D, F), bf16),
            pltpu.VMEM((256, 256), bf16),
            pltpu.VMEM((4, D), bf16),
            pltpu.VMEM((D,), bf16),
            pltpu.VMEM((F,), bf16),
            pltpu.VMEM((D,), bf16),
            pltpu.SemaphoreType.DMA((8,)),
            pltpu.SMEM((1,), jnp.int32),
            pltpu.VMEM((6, D, B), f32),
            pltpu.VMEM((D // 2, 2 * T), u32),
            pltpu.VMEM((D, T), f32),
            pltpu.VMEM((8, F), f32),
            pltpu.VMEM((128, 256), u32),
            pltpu.VMEM((D // 2, F), u32),
            pltpu.VMEM((D // 2, F), u32),
            pltpu.VMEM((NT, 9, D, B), f32),
            pltpu.VMEM((NT, 9, D, B), f32),
            pltpu.VMEM((3, 4, D, B), f32),
            pltpu.VMEM((2, D // 2, T), u32),
            pltpu.VMEM((2, T // 2, D), u32),
            pltpu.VMEM((2, D, T), f32),
        ],
        out_shape=jax.ShapeDtypeStruct((D, S), bf16),
        compiler_params=pltpu.CompilerParams(
            dimension_semantics=("arbitrary",), vmem_limit_bytes=110 * 1024 * 1024),
        name="h3mlp",
    )(qT, kT, vT, A_ssm_k, B_w1, B_w2.T, g, A_shift_k.T, A_ssm_D, B_b1, B_b2)
    return out.T[None]
```

```python
import functools

import numpy as np
import jax
import jax.numpy as jnp
import jax.experimental.pallas as pl
import jax.experimental.pallas.tpu as pltpu

S, D, F = 2048, 448, 1792
T = 256
NT = S // T
B = 128
EPS = 1e-5
f32, bf16, u32 = jnp.float32, jnp.bfloat16, jnp.uint32

_NT_DIMS = (((1,), (1,)), ((), ()))
_C0 = float(np.sqrt(2.0 / np.pi))
_C1 = _C0 * 0.044715
_DUR = {"a": 256, "b": 448, "I": 448, "X": 448, "K": 448}
_MLP_SEQ = "a a a a b a a b a a b a a b a a b a a b b".split()


def _dft_matrix():
    n = np.arange(256)[:, None].astype(np.float64)
    k = np.arange(128)[None, :].astype(np.float64)
    th = 2 * np.pi * (k + 0.5) * n / 256
    return np.concatenate([np.cos(th), -np.sin(th)], axis=1).astype(np.float32)


def _pack(x):
    return pltpu.bitcast(x.astype(bf16), u32)


def _unpack(x):
    return pltpu.bitcast(x, bf16)


def _fold8(a):
    r = a[0:8]
    for i in range(8, a.shape[0], 8):
        r = r + a[i:i + 8]
    return r


def _stats(s1, s2):
    m = jnp.sum(s1, axis=0, keepdims=True) * (1.0 / D)
    e2 = jnp.sum(s2, axis=0, keepdims=True) * (1.0 / D)
    return m, jnp.maximum(e2 - m * m, 0.0)


def _join(arrs):
    tiles = []
    for a in arrs:
        a = pltpu.bitcast(a, u32)
        tiles += [a[i:i + 8, j:j + B] for i in range(0, a.shape[0], 8) for j in range(0, a.shape[1], B)]
    d = tiles[0]
    for x in tiles[1:]:
        d = d | x
    return d


def _kernel(q_hbm, k_hbm, v_hbm, ssm_hbm, w1_hbm, w2_hbm, g_hbm, sh_hbm, d_hbm, b1_hbm, b2_hbm,
            o_ref,
            q_ref, k_ref, v_ref, ssm_ref, w1_ref, w2_ref, g_ref, sh_ref, d_ref, b1_ref, b2_ref,
            sem, z_ref,
            par_ref, w_ref, h_ref, b1b_ref, gu_ref, w1u_ref, w2u_ref,
            xs_ref, ks_ref, lraw_ref, kvb_ref, yn_ref, hres_ref):
    step_id = pl.program_id(0)
    Q, K_, V_, SS, W1, W2 = range(6)
    srcs = (q_hbm, k_hbm, v_hbm, ssm_hbm)
    dsts = (q_ref, k_ref, v_ref, ssm_ref)
    ctx = {}

    def copy(a, t, si):
        if a < 4:
            return pltpu.make_async_copy(srcs[a].at[:, pl.ds(t * T, T)], dsts[a].at[t], sem.at[si])
        src, dst = ((w1_hbm, w1_ref), (w2_hbm, w2_ref))[a - 4]
        return pltpu.make_async_copy(src.at[:, pl.ds(t * 256, 256)], dst.at[:, pl.ds(t * 256, 256)], sem.at[si])

    def start(batch):
        for a, t in batch[1]:
            copy(a, t, batch[0]).start()

    def wait(batch):
        for a, t in batch[1]:
            copy(a, t, batch[0]).wait()

    B1 = (1, [(K_, 0), (V_, 0), (SS, 0)])
    BQ = (2, [(Q, 0)])
    B2 = (3, [(W1, 0), (W1, 1), (W2, 0)])
    B3 = (4, [(K_, 1), (V_, 1), (SS, 1), (W1, 2), (W2, 1), (W1, 3)])
    B4 = (5, [(W2, 2), (W1, 4), (W2, 3), (W1, 5), (SS, 2), (Q, 1)])
    B5 = (6, [(W2, 4), (W1, 6), (W2, 5), (W2, 6), (K_, 2), (V_, 2)])
    B6 = (7, [(SS, 3), (Q, 2), (K_, 3), (V_, 3), (SS, 4)])

    def step_batch(t):
        return (t % 2, [(a, tt) for a, tt in ((Q, t), (K_, t + 1), (V_, t + 1), (SS, t + 2)) if tt < NT])

    def enter():
        ctx.clear()
        ctx["zero"] = z_ref[0]

    def link(dep, x):
        if dep is None:
            return x
        if x.shape not in ctx:
            ctx[x.shape] = jax.lax.broadcasted_iota(jnp.int32, x.shape, 1) < ctx["zero"]
        return jnp.where(ctx[x.shape], dep, x)

    def attach(x, deps):
        if not deps:
            return x
        parts = []
        pos = 0
        for r in sorted(deps):
            if 16 * r > pos:
                parts.append(x[pos:16 * r])
            blk = x[16 * r:16 * r + 16]
            t0 = _unpack(link(deps[r], pltpu.bitcast(blk[:, :B], u32)))
            parts.append(jnp.concatenate([t0, blk[:, B:]], axis=1))
            pos = 16 * r + 16
        if pos < x.shape[0]:
            parts.append(x[pos:])
        return jnp.concatenate(parts, axis=0)

    def gblk(b):
        return _unpack(gu_ref[b * 64:(b + 1) * 64, :])

    def dft(a):
        out = []
        for b in range(2):
            z = jnp.dot(a[:, b * B:(b + 1) * B], gblk(b), preferred_element_type=f32)
            out.append((z[:, :B], z[:, B:]))
        return out

    def kernel_dft(t):
        (c0, d0), (c1, d1) = dft(ssm_ref[t])
        if t == 0:
            c0 = c0 + par_ref[4]
        for i, a in enumerate((c0, d0, c1, d1)):
            lraw_ref[t % 3, i] = a

    def kernel_prep(t, r0, rc, l, chain=True):
        rows = slice(r0, r0 + rc)
        c0, d0, c1, d1 = (lraw_ref[t % 3, i, rows, :] for i in range(4))
        if t > 0:
            pc0, pd0, pc1, pd1 = (lraw_ref[(t - 1) % 3, i, rows, :] for i in range(4))
        else:
            pc0 = pd0 = pc1 = pd1 = None
        streams = ((c0, pc1, d0, pd1, -1), (c0, pc0, d0, pd0, 1), (c1, pc1, d1, pd1, 1))
        for p, (cc, pc, dd, pd, sg) in enumerate(streams):
            cc = link(l, cc)
            if pc is None:
                c, d = cc, dd
            else:
                c = cc + pc if sg > 0 else cc - pc
                d = dd + pd if sg > 0 else dd - pd
            e = d - c
            f = (link(e, c) if chain else c) + d
            l = f if chain else None
            ks_ref[t, 3 * p + 0, rows, :] = c
            ks_ref[t, 3 * p + 1, rows, :] = e
            ks_ref[t, 3 * p + 2, rows, :] = f
        return l

    def shift_kv(t, l=None, nchain=None, rc=16):
        lane = jax.lax.broadcasted_iota(jnp.int32, (rc // 2, B), 1)
        edge = [None] + [lane >= B - u for u in (1, 2, 3)]
        links = [None if l is None else pltpu.bitcast(l, u32)] * (nchain or 1)
        n = 0
        for r0 in range(0, D, rc):
            rows = slice(r0, r0 + rc)
            kp = pltpu.bitcast(k_ref[t, rows, :], u32)
            if t == 0:
                prev = jnp.zeros((rc // 2, B), u32)
            else:
                prev = pltpu.bitcast(k_ref[t - 1, rows, B:2 * B], u32)
            v = v_ref[t, rows, :].astype(f32)
            cols = [prev, kp[:, :B], kp[:, B:]]
            for c in (1, 2):
                cur = link(links[n % len(links)], cols[c])
                a = _unpack(cur).astype(f32) * par_ref[0, rows, :]
                for u in (1, 2, 3):
                    m = jnp.where(edge[u], cols[c - 1], cur)
                    a = a + _unpack(pltpu.roll(m, u, 1)).astype(f32) * par_ref[u, rows, :]
                out = _pack(a * v[:, (c - 1) * B:c * B])
                if nchain:
                    links[n % nchain] = out
                n += 1
                kvb_ref[t % 2, r0 // 2:(r0 + rc) // 2, (c - 1) * B:c * B] = out

    def kv_dft(t):
        (a0, b0), (a1, b1) = dft(_unpack(kvb_ref[t % 2]))
        s0 = a0 + b0
        s1 = a1 + b1
        for j, a in enumerate((s0 + s1, a0 + a1, b0 + b1, s1, a1, b1, s0, a0, b0)):
            xs_ref[t, j] = a

    def mac_rows(t, r0, rc, l, chain=True):
        rows = slice(r0, r0 + rc)
        lk = link if chain else (lambda dep, x: x)

        def term(j, u):
            return xs_ref[u, j, rows, :] * ks_ref[t - u, j, rows, :]

        def run(a, j, sign, first=0):
            for u in range(first, t + 1):
                a = a + term(j, u) if sign > 0 else a - term(j, u)
            return a

        r0_ = run(lk(l, term(0, 0)), 0, 1, 1)
        p1r = run(r0_, 2, -1)
        p1i = run(lk(p1r, r0_), 1, 1)
        r3 = run(lk(p1i, term(3, 0)), 3, 1, 1)
        w0r = run(p1r - r3, 5, 1)
        w0i = run(lk(w0r, p1i - r3), 4, -1)
        r6 = run(lk(w0i, term(6, 0)), 6, 1, 1)
        w1r = run(p1r + r6, 8, -1)
        w1i = run(lk(w1r, p1i + r6), 7, 1)
        w_ref[r0 // 2:(r0 + rc) // 2, :] = _pack(jnp.concatenate([w0r, w0i, w1r, w1i], axis=1))
        return w1i

    def mac_chain(t, kp_pre=None, kp_post=None):
        l = None
        for r0 in range(0, D, 16):
            if kp_pre is not None:
                l = kernel_prep(kp_pre, r0, 16, l)
            l = mac_rows(t, r0, 16, l)
            if kp_post is not None:
                l = kernel_prep(kp_post, r0, 16, l)

    def inverse_dft():
        ys = []
        for b in range(2):
            ys.append(jax.lax.dot_general(_unpack(w_ref[:, 2 * b * B:2 * (b + 1) * B]), gblk(b), _NT_DIMS,
                                          preferred_element_type=f32))
        return jnp.concatenate(ys, axis=1)

    def norms(t, get_y):
        s1 = s2 = None
        for r0 in range(0, D, 64):
            x = q_ref[t, r0:r0 + 64, :].astype(f32)
            a, b = _fold8(x), _fold8(x * x)
            s1 = a if s1 is None else s1 + a
            s2 = b if s2 is None else s2 + b
            yield _join([s1, s2])
        m, var = _stats(s1, s2)
        rq = jax.lax.rsqrt(var + EPS) * (1.0 / 128.0)
        mq = m * rq
        y = get_y()
        s1 = s2 = None
        for r0 in range(0, D, 32):
            rows = slice(r0, r0 + 32)
            x = q_ref[t, rows, :].astype(f32)
            h = x + (x * rq - mq) * y[rows]
            h_ref[rows, :] = h
            b2 = par_ref[5, rows, :]
            hres_ref[t % 2, rows, :] = (h + h) + jnp.concatenate([b2, b2], axis=1)
            a, b = _fold8(h), _fold8(h * h)
            s1 = a if s1 is None else s1 + a
            s2 = b if s2 is None else s2 + b
        yield None
        mh, vh = _stats(s1, s2)
        rh = jax.lax.rsqrt(vh + EPS)
        rz = jax.lax.rsqrt(vh * (rh * rh) + EPS)
        sc = rh * rz
        sh = (mh * rh) * rz
        for c in range(2):
            for r0 in range(0, D, B):
                rc = min(B, D - r0)
                hv = h_ref[pl.ds(pl.multiple_of(r0 + ctx["zero"], 8), rc), c * B:(c + 1) * B]
                yt = (hv * sc[:, c * B:(c + 1) * B] - sh[:, c * B:(c + 1) * B]).astype(bf16).T
                yn_ref[t % 2, c * 64:(c + 1) * 64, r0:r0 + rc] = pltpu.bitcast(yt, u32)
                if rc < B:
                    yt = jnp.concatenate([yt, yt], axis=1)
                yield _join([yt[0:16], yt[B - 16:B]])

    def mlp_up(t, c, deps, yn=None):
        f0, f1 = c * B, (c + 1) * B
        if t == 0:
            wv = w1_ref[:, f0:f1]
            w1u_ref[:, f0:f1] = pltpu.bitcast(wv, u32)
        else:
            wv = _unpack(w1u_ref[:, f0:f1])
        if yn is None:
            yn = _unpack(yn_ref[t % 2])
        x = jnp.dot(attach(yn, deps), wv, preferred_element_type=f32)
        x = x + jnp.concatenate([b1b_ref[:, f0:f1]] * (x.shape[0] // 8), axis=0)
        return x + x * jnp.tanh(x * (_C0 + _C1 * (x * x)))

    def mlp_down(t, hh, c, acc, deps):
        if t == 0:
            wv = w2_ref[:, c * 256:(c + 1) * 256]
            w2u_ref[:, c * 256:(c + 1) * 256] = pltpu.bitcast(wv, u32)
        else:
            wv = _unpack(w2u_ref[:, c * 256:(c + 1) * 256])
        return acc + jax.lax.dot_general(attach(wv, deps), hh.astype(bf16), _NT_DIMS, preferred_element_type=f32)

    def run_seq(tm, seq, special, add_tasks):
        t0s = []
        total = 0
        for op in seq:
            t0s.append(total)
            total += _DUR.get(op[0], 0)
        pts = [(t0s[m] + 16 * r, m, r) for m, op in enumerate(seq) if op in ("a", "b")
               for r in range(16 if op == "a" else 28)]
        tasks = {}

        def spread(fn, n, lo, hi):
            for k in range(n):
                when = lo + (hi - lo) * (k + 1) / n
                tasks[next((m, r) for (tp, m, r) in pts if tp >= when and (m, r) not in tasks)] = fn

        add_tasks(lambda op: t0s[seq.index(op)], total, spread)
        hh = {}
        acc = None
        na = nb = 0
        for m, op in enumerate(seq):
            deps = {r: tasks[(mm, r)]() for (mm, r) in sorted(tasks) if mm == m}
            if op == "a":
                hh[na] = mlp_up(tm, na, deps)
                na += 1
            elif op == "b":
                if acc is None:
                    acc = hres_ref[tm % 2]
                acc = mlp_down(tm, jnp.concatenate([hh[2 * nb], hh[2 * nb + 1]], axis=1), nb, acc, deps)
                nb += 1
            else:
                special[op]()
        o_ref[...] = (acc * 0.5).astype(o_ref.dtype)

    def step0():
        small = [pltpu.make_async_copy(a, b, sem.at[0]) for a, b in
                 ((sh_hbm, sh_ref), (d_hbm, d_ref), (b2_hbm, b2_ref), (b1_hbm, b1_ref), (g_hbm, g_ref))]
        for c in small:
            c.start()
        for b in (B1, BQ, B2, B3, B4, B5, B6):
            start(b)
        z_ref[0] = 0
        for c in small:
            c.wait()

        def col(r):
            return jnp.broadcast_to(r, (B, D)).T

        sh = sh_ref[...].astype(f32)
        for u in range(4):
            par_ref[u] = col(sh[u:u + 1])
        par_ref[4] = col(d_ref[...].reshape(1, D).astype(f32))
        par_ref[5] = col(b2_ref[...].reshape(1, D).astype(f32) * 2.0)
        gu_ref[...] = pltpu.bitcast(g_ref[...], u32)
        b1b_ref[...] = jnp.broadcast_to(b1_ref[...].reshape(1, F).astype(f32), (8, F))
        wait(B1)
        kernel_dft(0)
        shift_kv(0, rc=D)
        kv_dft(0)
        for r0 in range(0, D, 32):
            kernel_prep(0, r0, 32, None, chain=False)
            mac_rows(0, r0, 32, None, chain=False)

    def step1():
        enter()
        ybox = []
        ln1 = norms(1, lambda: ybox[0])

        def finish_tile0():
            y = inverse_dft()
            for _ in norms(0, lambda: y):
                pass

        special = {
            "wq": lambda: wait(BQ),
            "I0": finish_tile0,
            "w2": lambda: wait(B2),
            "w3": lambda: wait(B3),
            "K1": lambda: (kernel_dft(1), kernel_prep(1, 0, D, None, chain=False)),
            "v1": lambda: shift_kv(1, None, 6),
            "w4": lambda: wait(B4),
            "X1": lambda: kv_dft(1),
            "K2": lambda: (mac_chain(1), kernel_dft(2)),
            "w5": lambda: wait(B5),
            "I1": lambda: (ybox.append(inverse_dft()), next(ln1)),
            "e": lambda: shift_kv(2, ybox[0][D - 8:D, 0:B], 8),
        }
        seq = "wq I0 w2 a a a a b w3 K1 a a b a a v1 w4 X1 b a a b a a K2 w5 I1 b a a b b e".split()

        def add_tasks(at, total, spread):
            t_y = at("I1") + 448
            spread(lambda: next(ln1), 7, at("X1") + 448, at("K2") - 100)
            spread(lambda: next(ln1), 8, t_y + 500, min(t_y + 1000, total - 150))

        run_seq(0, seq, special, add_tasks)

    def step(t):
        enter()
        nxt = t + 1 < NT
        has_k = t + 2 < NT
        wait(B6 if t == 2 else step_batch(t))
        if nxt:
            start(step_batch(t + 1))
        kp_pre = t if t in (2, NT - 1) else None
        kp_post = t + 1 if t + 1 < NT - 1 else None
        t_mac = (100 + 28 * (18 * (t + 1) + 14 + (24 if kp_pre else 0) + (24 if kp_post else 0)) * 1.05
                 - (448 if has_k else 0))
        tt = 0
        pos = len(_MLP_SEQ)
        for m, op in enumerate(_MLP_SEQ):
            if tt >= t_mac:
                pos = m
                break
            tt += _DUR[op]
        seq = ((["K3"] if t == 2 else []) + ["X"] + _MLP_SEQ[:pos] + ["M"] + (["K"] if has_k else [])
               + ["I"] + _MLP_SEQ[pos:] + ["e"])
        ybox = []
        ln = norms(t, lambda: ybox[0])
        info = {}

        def add_tasks(at, total, spread):
            t_y = at("I") + 448
            spread(lambda: next(ln), 7, at("X") + 448, at("I") - 100 - (448 if has_k else 0))
            spread(lambda: next(ln), 8, t_y + 500, min(t_y + 1000, total - 150))
            info["left"] = total - t_y - 1000

        def finish():
            if nxt:
                nchain = max(4, min(8, int(np.ceil(56 * 135 / max(info["left"], 1)))))
                shift_kv(t + 1, ybox[0][D - 8:D, 0:B], nchain)

        special = {
            "K3": lambda: kernel_dft(3),
            "X": lambda: kv_dft(t),
            "M": lambda: mac_chain(t, kp_pre, kp_post),
            "K": lambda: kernel_dft(t + 2),
            "I": lambda: (ybox.append(inverse_dft()), next(ln)),
            "e": finish,
        }
        run_seq(t - 1, seq, special, add_tasks)

    def last_step():
        t = NT - 1

        def body(hf, carry):
            col = pl.ds(pl.multiple_of(hf * B, B), B)
            yn = _unpack(yn_ref[t % 2, pl.ds(pl.multiple_of(hf * 64, 64), 64), :])
            acc = hres_ref[t % 2, :, col]
            hh = {}
            na = nb = 0
            for op in "a a a a a a a a b a a a a b a a b b".split():
                if op == "a":
                    hh[na] = mlp_up(t, na, {}, yn)
                    na += 1
                    continue
                k0 = 4 * nb
                k1 = min(k0 + 4, F // B)
                hcat = jnp.concatenate([hh[k] for k in range(k0, k1)], axis=1).astype(bf16)
                mrows = D if k1 - k0 == 4 else D // 2
                parts = []
                for m0 in range(0, D, mrows):
                    wv = _unpack(w2u_ref[m0 // 2:(m0 + mrows) // 2, k0 * B:k1 * B])
                    parts.append(acc[m0:m0 + mrows]
                                 + jax.lax.dot_general(wv, hcat, _NT_DIMS, preferred_element_type=f32))
                acc = parts[0] if len(parts) == 1 else jnp.concatenate(parts, axis=0)
                nb += 1
            o_ref[:, col] = (acc * 0.5).astype(o_ref.dtype)
            return carry

        jax.lax.fori_loop(0, 2, body, 0)

    fns = [step0, step1] + [functools.partial(step, i) for i in range(2, NT)] + [last_step]
    for i, fn in enumerate(fns):
        pl.when(step_id == i)(fn)


@jax.jit
def pallas_sequential_preLN__ssm_conv_h3__mixer_channel_mlp__prompt_kernel(
        A_q, A_k, A_v, A_shift_k, A_ssm_k, A_ssm_D, B_x, B_w1, B_b1, B_w2, B_b2):
    del B_x
    qT = jnp.transpose(A_q[0])
    kT = jnp.transpose(A_k[0])
    vT = jnp.transpose(A_v[0])
    g = jnp.asarray(_dft_matrix(), dtype=bf16)
    out = pl.pallas_call(
        _kernel,
        grid=(NT + 1,),
        in_specs=[pl.BlockSpec(memory_space=pl.ANY)] * 11,
        out_specs=pl.BlockSpec((D, T), lambda i: (0, jnp.maximum(i - 1, 0))),
        scratch_shapes=[
            pltpu.VMEM((NT, D, T), bf16),
            pltpu.VMEM((NT, D, T), bf16),
            pltpu.VMEM((NT, D, T), bf16),
            pltpu.VMEM((NT, D, T), bf16),
            pltpu.VMEM((D, F), bf16),
            pltpu.VMEM((D, F), bf16),
            pltpu.VMEM((256, 256), bf16),
            pltpu.VMEM((4, D), bf16),
            pltpu.VMEM((D,), bf16),
            pltpu.VMEM((F,), bf16),
            pltpu.VMEM((D,), bf16),
            pltpu.SemaphoreType.DMA((8,)),
            pltpu.SMEM((1,), jnp.int32),
            pltpu.VMEM((6, D, B), f32),
            pltpu.VMEM((D // 2, 2 * T), u32),
            pltpu.VMEM((D, T), f32),
            pltpu.VMEM((8, F), f32),
            pltpu.VMEM((128, 256), u32),
            pltpu.VMEM((D // 2, F), u32),
            pltpu.VMEM((D // 2, F), u32),
            pltpu.VMEM((NT, 9, D, B), f32),
            pltpu.VMEM((NT, 9, D, B), f32),
            pltpu.VMEM((3, 4, D, B), f32),
            pltpu.VMEM((2, D // 2, T), u32),
            pltpu.VMEM((2, T // 2, D), u32),
            pltpu.VMEM((2, D, T), f32),
        ],
        out_shape=jax.ShapeDtypeStruct((D, S), bf16),
        compiler_params=pltpu.CompilerParams(
            dimension_semantics=("arbitrary",), vmem_limit_bytes=110 * 1024 * 1024),
        name="h3mlp",
    )(qT, kT, vT, A_ssm_k, B_w1, B_w2.T, g, A_shift_k.T, A_ssm_D, B_b1, B_b2)
    return out.T[None]
```

```python
import functools

import numpy as np
import jax
import jax.numpy as jnp
import jax.experimental.pallas as pl
import jax.experimental.pallas.tpu as pltpu

S, D, F = 2048, 448, 1792
T = 256
NT = S // T
B = 128
EPS = 1e-5
f32, bf16, u32 = jnp.float32, jnp.bfloat16, jnp.uint32

_NT_DIMS = (((1,), (1,)), ((), ()))
_C0 = float(np.sqrt(2.0 / np.pi))
_C1 = _C0 * 0.044715
_DUR = {"a": 256, "b": 448, "I": 448, "X": 448, "K": 448}
_MLP_SEQ = "a a a a b a a b a a b a a b a a b a a b b".split()


def _dft_matrix():
    n = np.arange(256)[:, None].astype(np.float64)
    k = np.arange(128)[None, :].astype(np.float64)
    th = 2 * np.pi * (k + 0.5) * n / 256
    return np.concatenate([np.cos(th), -np.sin(th)], axis=1).astype(np.float32)


def _pack(x):
    return pltpu.bitcast(x.astype(bf16), u32)


def _unpack(x):
    return pltpu.bitcast(x, bf16)


def _fold8(a):
    r = a[0:8]
    for i in range(8, a.shape[0], 8):
        r = r + a[i:i + 8]
    return r


def _stats(s1, s2):
    m = jnp.sum(s1, axis=0, keepdims=True) * (1.0 / D)
    e2 = jnp.sum(s2, axis=0, keepdims=True) * (1.0 / D)
    return m, jnp.maximum(e2 - m * m, 0.0)


def _join(arrs):
    tiles = []
    for a in arrs:
        a = pltpu.bitcast(a, u32)
        tiles += [a[i:i + 8, j:j + B] for i in range(0, a.shape[0], 8) for j in range(0, a.shape[1], B)]
    d = tiles[0]
    for x in tiles[1:]:
        d = d | x
    return d


def _kernel(q_hbm, k_hbm, v_hbm, ssm_hbm, w1_hbm, w2_hbm, g_hbm, sh_hbm, d_hbm, b1_hbm, b2_hbm,
            o_ref,
            q_ref, k_ref, v_ref, ssm_ref, w1_ref, w2_ref, g_ref, sh_ref, d_ref, b1_ref, b2_ref,
            sem, z_ref,
            par_ref, w_ref, h_ref, b1b_ref, gu_ref, w1u_ref, w2u_ref,
            xs_ref, ks_ref, lraw_ref, kvb_ref, yn_ref, hres_ref):
    step_id = pl.program_id(0)
    Q, K_, V_, SS, W1, W2 = range(6)
    srcs = (q_hbm, k_hbm, v_hbm, ssm_hbm)
    dsts = (q_ref, k_ref, v_ref, ssm_ref)
    ctx = {}

    def copy(a, t, si):
        if a < 4:
            return pltpu.make_async_copy(srcs[a].at[:, pl.ds(t * T, T)], dsts[a].at[t], sem.at[si])
        src, dst = ((w1_hbm, w1_ref), (w2_hbm, w2_ref))[a - 4]
        return pltpu.make_async_copy(src.at[:, pl.ds(t * 256, 256)], dst.at[:, pl.ds(t * 256, 256)], sem.at[si])

    def start(batch):
        for a, t in batch[1]:
            copy(a, t, batch[0]).start()

    def wait(batch):
        for a, t in batch[1]:
            copy(a, t, batch[0]).wait()

    B1 = (1, [(K_, 0), (V_, 0), (SS, 0)])
    BQ = (2, [(Q, 0)])
    B2 = (3, [(W1, 0), (W1, 1), (W2, 0)])
    B3 = (4, [(K_, 1), (V_, 1), (SS, 1), (W1, 2), (W2, 1), (W1, 3)])
    B4 = (5, [(W2, 2), (W1, 4), (W2, 3), (W1, 5), (SS, 2), (Q, 1)])
    B5 = (6, [(W2, 4), (W1, 6), (W2, 5), (W2, 6), (K_, 2), (V_, 2)])
    B6 = (7, [(SS, 3), (Q, 2), (K_, 3), (V_, 3), (SS, 4)])

    def step_batch(t):
        return (t % 2, [(a, tt) for a, tt in ((Q, t), (K_, t + 1), (V_, t + 1), (SS, t + 2)) if tt < NT])

    def enter():
        ctx.clear()
        ctx["zero"] = z_ref[0]

    def link(dep, x):
        if dep is None:
            return x
        if x.shape not in ctx:
            ctx[x.shape] = jax.lax.broadcasted_iota(jnp.int32, x.shape, 1) < ctx["zero"]
        return jnp.where(ctx[x.shape], dep, x)

    def attach(x, deps):
        if not deps:
            return x
        parts = []
        pos = 0
        for r in sorted(deps):
            if 16 * r > pos:
                parts.append(x[pos:16 * r])
            blk = x[16 * r:16 * r + 16]
            t0 = _unpack(link(deps[r], pltpu.bitcast(blk[:, :B], u32)))
            parts.append(jnp.concatenate([t0, blk[:, B:]], axis=1))
            pos = 16 * r + 16
        if pos < x.shape[0]:
            parts.append(x[pos:])
        return jnp.concatenate(parts, axis=0)

    def gblk(b):
        return _unpack(gu_ref[b * 64:(b + 1) * 64, :])

    def dft(a):
        out = []
        for b in range(2):
            z = jnp.dot(a[:, b * B:(b + 1) * B], gblk(b), preferred_element_type=f32)
            out.append((z[:, :B], z[:, B:]))
        return out

    def kernel_dft(t):
        (c0, d0), (c1, d1) = dft(ssm_ref[t])
        if t == 0:
            c0 = c0 + par_ref[4]
        for i, a in enumerate((c0, d0, c1, d1)):
            lraw_ref[t % 3, i] = a

    def kernel_prep(t, r0, rc, l, chain=True):
        rows = slice(r0, r0 + rc)
        cur = lraw_ref[t % 3, :, rows, :]
        c0, d0, c1, d1 = (cur[i] for i in range(4))
        if t > 0:
            prv = lraw_ref[(t - 1) % 3, :, rows, :]
            pc0, pd0, pc1, pd1 = (prv[i] for i in range(4))
        else:
            pc0 = pd0 = pc1 = pd1 = None
        streams = ((c0, pc1, d0, pd1, -1), (c0, pc0, d0, pd0, 1), (c1, pc1, d1, pd1, 1))
        outs = []
        for (cc, pc, dd, pd, sg) in streams:
            cc = link(l, cc)
            if pc is None:
                c, d = cc, dd
            else:
                c = cc + pc if sg > 0 else cc - pc
                d = dd + pd if sg > 0 else dd - pd
            e = d - c
            f = (link(e, c) if chain else c) + d
            l = f if chain else None
            outs += [c, e, f]
        ks_ref[t, :, rows, :] = jnp.stack(outs)
        return l

    def shift_kv(t, l=None, nchain=None, rc=16):
        lane = jax.lax.broadcasted_iota(jnp.int32, (rc // 2, B), 1)
        edge = [None] + [lane >= B - u for u in (1, 2, 3)]
        links = [None if l is None else pltpu.bitcast(l, u32)] * (nchain or 1)
        n = 0
        for r0 in range(0, D, rc):
            rows = slice(r0, r0 + rc)
            kp = pltpu.bitcast(k_ref[t, rows, :], u32)
            if t == 0:
                prev = jnp.zeros((rc // 2, B), u32)
            else:
                prev = pltpu.bitcast(k_ref[t - 1, rows, B:2 * B], u32)
            v = v_ref[t, rows, :].astype(f32)
            cols = [prev, kp[:, :B], kp[:, B:]]
            taps = par_ref[0:4, rows, :]
            for c in (1, 2):
                cur = link(links[n % len(links)], cols[c])
                a = _unpack(cur).astype(f32) * taps[0]
                for u in (1, 2, 3):
                    m = jnp.where(edge[u], cols[c - 1], cur)
                    a = a + _unpack(pltpu.roll(m, u, 1)).astype(f32) * taps[u]
                out = _pack(a * v[:, (c - 1) * B:c * B])
                if nchain:
                    links[n % nchain] = out
                n += 1
                kvb_ref[t % 2, r0 // 2:(r0 + rc) // 2, (c - 1) * B:c * B] = out

    def kv_dft(t):
        (a0, b0), (a1, b1) = dft(_unpack(kvb_ref[t % 2]))
        s0 = a0 + b0
        s1 = a1 + b1
        for j, a in enumerate((s0 + s1, a0 + a1, b0 + b1, s1, a1, b1, s0, a0, b0)):
            xs_ref[t, j] = a

    def mac_rows(t, r0, rc, l, chain=True):
        rows = slice(r0, r0 + rc)
        lk = link if chain else (lambda dep, x: x)

        prod = [xs_ref[u, :, rows, :] * ks_ref[t - u, :, rows, :] for u in range(t + 1)]

        def term(j, u):
            return prod[u][j]

        def run(a, j, sign, first=0):
            for u in range(first, t + 1):
                a = a + term(j, u) if sign > 0 else a - term(j, u)
            return a

        r0_ = run(lk(l, term(0, 0)), 0, 1, 1)
        p1r = run(r0_, 2, -1)
        p1i = run(lk(p1r, r0_), 1, 1)
        r3 = run(lk(p1i, term(3, 0)), 3, 1, 1)
        w0r = run(p1r - r3, 5, 1)
        w0i = run(lk(w0r, p1i - r3), 4, -1)
        r6 = run(lk(w0i, term(6, 0)), 6, 1, 1)
        w1r = run(p1r + r6, 8, -1)
        w1i = run(lk(w1r, p1i + r6), 7, 1)
        w_ref[r0 // 2:(r0 + rc) // 2, :] = _pack(jnp.concatenate([w0r, w0i, w1r, w1i], axis=1))
        return w1i

    def mac_chain(t, kp_pre=None, kp_post=None):
        l = None
        for r0 in range(0, D, 16):
            if kp_pre is not None:
                l = kernel_prep(kp_pre, r0, 16, l)
            l = mac_rows(t, r0, 16, l)
            if kp_post is not None:
                l = kernel_prep(kp_post, r0, 16, l)

    def inverse_dft():
        ys = []
        for b in range(2):
            ys.append(jax.lax.dot_general(_unpack(w_ref[:, 2 * b * B:2 * (b + 1) * B]), gblk(b), _NT_DIMS,
                                          preferred_element_type=f32))
        return jnp.concatenate(ys, axis=1)

    def norms(t, get_y):
        s1 = s2 = None
        for r0 in range(0, D, 64):
            x = q_ref[t, r0:r0 + 64, :].astype(f32)
            a, b = _fold8(x), _fold8(x * x)
            s1 = a if s1 is None else s1 + a
            s2 = b if s2 is None else s2 + b
            yield _join([s1, s2])
        m, var = _stats(s1, s2)
        rq = jax.lax.rsqrt(var + EPS) * (1.0 / 128.0)
        mq = m * rq
        y = get_y()
        s1 = s2 = None
        for r0 in range(0, D, 32):
            rows = slice(r0, r0 + 32)
            x = q_ref[t, rows, :].astype(f32)
            h = x + (x * rq - mq) * y[rows]
            h_ref[rows, :] = h
            b2 = par_ref[5, rows, :]
            hres_ref[t % 2, rows, :] = (h + h) + jnp.concatenate([b2, b2], axis=1)
            a, b = _fold8(h), _fold8(h * h)
            s1 = a if s1 is None else s1 + a
            s2 = b if s2 is None else s2 + b
        yield None
        mh, vh = _stats(s1, s2)
        rh = jax.lax.rsqrt(vh + EPS)
        rz = jax.lax.rsqrt(vh * (rh * rh) + EPS)
        sc = rh * rz
        sh = (mh * rh) * rz
        for c in range(2):
            for r0 in range(0, D, B):
                rc = min(B, D - r0)
                hv = h_ref[r0:r0 + rc, c * B:(c + 1) * B]
                yt = (hv * sc[:, c * B:(c + 1) * B] - sh[:, c * B:(c + 1) * B]).astype(bf16).T
                yn_ref[t % 2, c * 64:(c + 1) * 64, r0:r0 + rc] = pltpu.bitcast(yt, u32)
                if rc < B:
                    yt = jnp.concatenate([yt, yt], axis=1)
                yield _join([yt[0:16], yt[B - 16:B]])

    def mlp_up(t, c, deps, yn=None):
        f0, f1 = c * B, (c + 1) * B
        if t == 0:
            wv = w1_ref[:, f0:f1]
            w1u_ref[:, f0:f1] = pltpu.bitcast(wv, u32)
        else:
            wv = _unpack(w1u_ref[:, f0:f1])
        if yn is None:
            yn = _unpack(yn_ref[t % 2])
        x = jnp.dot(attach(yn, deps), wv, preferred_element_type=f32)
        x = x + jnp.concatenate([b1b_ref[:, f0:f1]] * (x.shape[0] // 8), axis=0)
        return x + x * jnp.tanh(x * (_C0 + _C1 * (x * x)))

    def mlp_down(t, hh, c, acc, deps):
        if t == 0:
            wv = w2_ref[:, c * 256:(c + 1) * 256]
            w2u_ref[:, c * 256:(c + 1) * 256] = pltpu.bitcast(wv, u32)
        else:
            wv = _unpack(w2u_ref[:, c * 256:(c + 1) * 256])
        return acc + jax.lax.dot_general(attach(wv, deps), hh.astype(bf16), _NT_DIMS, preferred_element_type=f32)

    def run_seq(tm, seq, special, add_tasks):
        t0s = []
        total = 0
        for op in seq:
            t0s.append(total)
            total += _DUR.get(op[0], 0)
        pts = [(t0s[m] + 16 * r, m, r) for m, op in enumerate(seq) if op in ("a", "b")
               for r in range(16 if op == "a" else 28)]
        tasks = {}

        def spread(fn, n, lo, hi):
            for k in range(n):
                when = lo + (hi - lo) * (k + 1) / n
                tasks[next((m, r) for (tp, m, r) in pts if tp >= when and (m, r) not in tasks)] = fn

        add_tasks(lambda op: t0s[seq.index(op)], total, spread)
        hh = {}
        acc = None
        na = nb = 0
        for m, op in enumerate(seq):
            deps = {r: tasks[(mm, r)]() for (mm, r) in sorted(tasks) if mm == m}
            if op == "a":
                hh[na] = mlp_up(tm, na, deps)
                na += 1
            elif op == "b":
                if acc is None:
                    acc = hres_ref[tm % 2]
                acc = mlp_down(tm, jnp.concatenate([hh[2 * nb], hh[2 * nb + 1]], axis=1), nb, acc, deps)
                nb += 1
            else:
                special[op]()
        o_ref[...] = (acc * 0.5).astype(o_ref.dtype)

    def step0():
        small = [pltpu.make_async_copy(a, b, sem.at[0]) for a, b in
                 ((sh_hbm, sh_ref), (d_hbm, d_ref), (b2_hbm, b2_ref), (b1_hbm, b1_ref), (g_hbm, g_ref))]
        for c in small:
            c.start()
        for b in (B1, BQ, B2, B3, B4, B5, B6):
            start(b)
        z_ref[0] = 0
        for c in small:
            c.wait()

        def col(r):
            return jnp.broadcast_to(r, (B, D)).T

        sh = sh_ref[...].astype(f32)
        for u in range(4):
            par_ref[u] = col(sh[u:u + 1])
        par_ref[4] = col(d_ref[...].reshape(1, D).astype(f32))
        par_ref[5] = col(b2_ref[...].reshape(1, D).astype(f32) * 2.0)
        gu_ref[...] = pltpu.bitcast(g_ref[...], u32)
        b1b_ref[...] = jnp.broadcast_to(b1_ref[...].reshape(1, F).astype(f32), (8, F))
        wait(B1)
        kernel_dft(0)
        shift_kv(0, rc=D)
        kv_dft(0)
        for r0 in range(0, D, 32):
            kernel_prep(0, r0, 32, None, chain=False)
            mac_rows(0, r0, 32, None, chain=False)

    def step1():
        enter()
        ybox = []
        ln1 = norms(1, lambda: ybox[0])

        def finish_tile0():
            y = inverse_dft()
            for _ in norms(0, lambda: y):
                pass

        special = {
            "wq": lambda: wait(BQ),
            "I0": finish_tile0,
            "w2": lambda: wait(B2),
            "w3": lambda: wait(B3),
            "K1": lambda: (kernel_dft(1), kernel_prep(1, 0, D, None, chain=False)),
            "v1": lambda: shift_kv(1, None, 6),
            "w4": lambda: wait(B4),
            "X1": lambda: kv_dft(1),
            "K2": lambda: (mac_chain(1), kernel_dft(2)),
            "w5": lambda: wait(B5),
            "I1": lambda: (ybox.append(inverse_dft()), next(ln1)),
            "e": lambda: shift_kv(2, ybox[0][D - 8:D, 0:B], 8),
        }
        seq = "wq I0 w2 a a a a b w3 K1 a a b a a v1 w4 X1 b a a b a a K2 w5 I1 b a a b b e".split()

        def add_tasks(at, total, spread):
            t_y = at("I1") + 448
            spread(lambda: next(ln1), 7, at("X1") + 448, at("K2") - 100)
            spread(lambda: next(ln1), 8, t_y + 500, min(t_y + 1000, total - 150))

        run_seq(0, seq, special, add_tasks)

    def step(t):
        enter()
        nxt = t + 1 < NT
        has_k = t + 2 < NT
        wait(B6 if t == 2 else step_batch(t))
        if nxt:
            start(step_batch(t + 1))
        kp_pre = t if t in (2, NT - 1) else None
        kp_post = t + 1 if t + 1 < NT - 1 else None
        t_mac = (100 + 28 * (18 * (t + 1) + 14 + (24 if kp_pre else 0) + (24 if kp_post else 0)) * 1.05
                 - (448 if has_k else 0))
        tt = 0
        pos = len(_MLP_SEQ)
        for m, op in enumerate(_MLP_SEQ):
            if tt >= t_mac:
                pos = m
                break
            tt += _DUR[op]
        seq = ((["K3"] if t == 2 else []) + ["X"] + _MLP_SEQ[:pos] + ["M"] + (["K"] if has_k else [])
               + ["I"] + _MLP_SEQ[pos:] + ["e"])
        ybox = []
        ln = norms(t, lambda: ybox[0])
        info = {}

        def add_tasks(at, total, spread):
            t_y = at("I") + 448
            spread(lambda: next(ln), 7, at("X") + 448, at("I") - 100 - (448 if has_k else 0))
            spread(lambda: next(ln), 8, t_y + 500, min(t_y + 1000, total - 150))
            info["left"] = total - t_y - 1000

        def finish():
            if nxt:
                nchain = max(4, min(8, int(np.ceil(56 * 135 / max(info["left"], 1)))))
                shift_kv(t + 1, ybox[0][D - 8:D, 0:B], nchain)

        special = {
            "K3": lambda: kernel_dft(3),
            "X": lambda: kv_dft(t),
            "M": lambda: mac_chain(t, kp_pre, kp_post),
            "K": lambda: kernel_dft(t + 2),
            "I": lambda: (ybox.append(inverse_dft()), next(ln)),
            "e": finish,
        }
        run_seq(t - 1, seq, special, add_tasks)

    def last_step():
        t = NT - 1

        def body(hf, carry):
            col = pl.ds(pl.multiple_of(hf * B, B), B)
            yn = _unpack(yn_ref[t % 2, pl.ds(pl.multiple_of(hf * 64, 64), 64), :])
            acc = hres_ref[t % 2, :, col]
            hh = {}
            na = nb = 0
            for op in "a a a a a a a a b a a a a b a a b b".split():
                if op == "a":
                    hh[na] = mlp_up(t, na, {}, yn)
                    na += 1
                    continue
                k0 = 4 * nb
                k1 = min(k0 + 4, F // B)
                hcat = jnp.concatenate([hh[k] for k in range(k0, k1)], axis=1).astype(bf16)
                mrows = D if k1 - k0 == 4 else D // 2
                parts = []
                for m0 in range(0, D, mrows):
                    wv = _unpack(w2u_ref[m0 // 2:(m0 + mrows) // 2, k0 * B:k1 * B])
                    parts.append(acc[m0:m0 + mrows]
                                 + jax.lax.dot_general(wv, hcat, _NT_DIMS, preferred_element_type=f32))
                acc = parts[0] if len(parts) == 1 else jnp.concatenate(parts, axis=0)
                nb += 1
            o_ref[:, col] = (acc * 0.5).astype(o_ref.dtype)
            return carry

        jax.lax.fori_loop(0, 2, body, 0)

    fns = [step0, step1] + [functools.partial(step, i) for i in range(2, NT)] + [last_step]
    for i, fn in enumerate(fns):
        pl.when(step_id == i)(fn)


@jax.jit
def pallas_sequential_preLN__ssm_conv_h3__mixer_channel_mlp__prompt_kernel(
        A_q, A_k, A_v, A_shift_k, A_ssm_k, A_ssm_D, B_x, B_w1, B_b1, B_w2, B_b2):
    del B_x
    qT = jnp.transpose(A_q[0])
    kT = jnp.transpose(A_k[0])
    vT = jnp.transpose(A_v[0])
    g = jnp.asarray(_dft_matrix(), dtype=bf16)
    out = pl.pallas_call(
        _kernel,
        grid=(NT + 1,),
        in_specs=[pl.BlockSpec(memory_space=pl.ANY)] * 11,
        out_specs=pl.BlockSpec((D, T), lambda i: (0, jnp.maximum(i - 1, 0))),
        scratch_shapes=[
            pltpu.VMEM((NT, D, T), bf16),
            pltpu.VMEM((NT, D, T), bf16),
            pltpu.VMEM((NT, D, T), bf16),
            pltpu.VMEM((NT, D, T), bf16),
            pltpu.VMEM((D, F), bf16),
            pltpu.VMEM((D, F), bf16),
            pltpu.VMEM((256, 256), bf16),
            pltpu.VMEM((4, D), bf16),
            pltpu.VMEM((D,), bf16),
            pltpu.VMEM((F,), bf16),
            pltpu.VMEM((D,), bf16),
            pltpu.SemaphoreType.DMA((8,)),
            pltpu.SMEM((1,), jnp.int32),
            pltpu.VMEM((6, D, B), f32),
            pltpu.VMEM((D // 2, 2 * T), u32),
            pltpu.VMEM((D, T), f32),
            pltpu.VMEM((8, F), f32),
            pltpu.VMEM((128, 256), u32),
            pltpu.VMEM((D // 2, F), u32),
            pltpu.VMEM((D // 2, F), u32),
            pltpu.VMEM((NT, 9, D, B), f32),
            pltpu.VMEM((NT, 9, D, B), f32),
            pltpu.VMEM((3, 4, D, B), f32),
            pltpu.VMEM((2, D // 2, T), u32),
            pltpu.VMEM((2, T // 2, D), u32),
            pltpu.VMEM((2, D, T), f32),
        ],
        out_shape=jax.ShapeDtypeStruct((D, S), bf16),
        compiler_params=pltpu.CompilerParams(
            dimension_semantics=("arbitrary",), vmem_limit_bytes=110 * 1024 * 1024),
        name="h3mlp",
    )(qT, kT, vT, A_ssm_k, B_w1, B_w2.T, g, A_shift_k.T, A_ssm_D, B_b1, B_b2)
    return out.T[None]
```
